```python
import os as _os
_os.environ.setdefault("JAX_PLATFORMS", "cpu")
import jax
import jax.numpy as jnp

def _softmax(x, axis=-1):
    return jax.nn.softmax(x, axis=axis)
def _gelu(x):
    return jax.nn.gelu(x, approximate=True)
def _silu(x):
    return jax.nn.silu(x)
def _sigmoid(x):
    return jax.nn.sigmoid(x)
def _layernorm(x, axis=-1, eps=1e-5):
    m = jnp.mean(x, axis=axis, keepdims=True)
    v = jnp.var(x, axis=axis, keepdims=True)
    return (x - m) / jnp.sqrt(v + eps)
def _scatter_add(tgt, idx, src, axis=0):
    return tgt.at[idx].add(src)
def _segment_sum(src, seg, n):
    return jax.ops.segment_sum(src, seg, n)
class _Rng:
    def __init__(self, key):
        self._k = key
    def _next(self):
        self._k, sub = jax.random.split(self._k)
        return sub
    def normal(self, shape):
        return jax.random.normal(self._next(), shape, dtype=jnp.bfloat16)
    def randint(self, lo, hi, shape):
        return jax.random.randint(self._next(), shape, lo, hi, dtype=jnp.int32)
    def uniform(self, shape, lo=0.0, hi=1.0):
        return jax.random.uniform(self._next(), shape, jnp.bfloat16, lo, hi)
    def permutation(self, n):
        return jax.random.permutation(self._next(), n)


kernel_name = 'gated_mix__ssm_conv_h3__ssm_conv_h3__prompt'

def setup_inputs():
    _rng = _Rng(jax.random.key(int.from_bytes(__import__("os").urandom(4), "little")))
    _w = (lambda a: (lambda t: t.astype(jnp.bfloat16) if jnp.issubdtype(t.dtype, jnp.floating) else t)(jnp.asarray(a)))
    def _A_setup():
        B, S, D = 1, 2048, 640
        ks = 4
        return {
            "q": _w((lambda *s: _rng.normal(s) * 0.05)(B, S, D)),
            "k": _w((lambda *s: _rng.normal(s) * 0.05)(B, S, D)),
            "v": _w((lambda *s: _rng.normal(s) * 0.05)(B, S, D)),
            "shift_k": _w((lambda *s: _rng.normal(s) * 0.05)(D, ks) * 0.5),
            "ssm_k": _w((lambda *s: _rng.normal(s) * 0.05)(D, S) * (1.0 / S ** 0.5)),
            "ssm_D": _w((lambda *s: _rng.normal(s) * 0.05)(D)),
        }
    _A_in = _A_setup()

    def _B_setup():
        B, S, D = 1, 2048, 640
        ks = 4
        return {
            "q": _w((lambda *s: _rng.normal(s) * 0.05)(B, S, D)),
            "k": _w((lambda *s: _rng.normal(s) * 0.05)(B, S, D)),
            "v": _w((lambda *s: _rng.normal(s) * 0.05)(B, S, D)),
            "shift_k": _w((lambda *s: _rng.normal(s) * 0.05)(D, ks) * 0.5),
            "ssm_k": _w((lambda *s: _rng.normal(s) * 0.05)(D, S) * (1.0 / S ** 0.5)),
            "ssm_D": _w((lambda *s: _rng.normal(s) * 0.05)(D)),
        }
    _B_in = _B_setup()

    return {
        "A_q": _A_in["q"],
        "A_k": _A_in["k"],
        "A_v": _A_in["v"],
        "A_shift_k": _A_in["shift_k"],
        "A_ssm_k": _A_in["ssm_k"],
        "A_ssm_D": _A_in["ssm_D"],
        "B_q": _B_in["q"],
        "B_k": _B_in["k"],
        "B_v": _B_in["v"],
        "B_shift_k": _B_in["shift_k"],
        "B_ssm_k": _B_in["ssm_k"],
        "B_ssm_D": _B_in["ssm_D"],
        "gate_w": _w((lambda *s: _rng.normal(s) * 0.05)(640) * 16.0),
    }

def reference(A_q, A_k, A_v, A_shift_k, A_ssm_k, A_ssm_D, B_q, B_k, B_v, B_shift_k, B_ssm_k, B_ssm_D, gate_w):
    def _A_ref(q, k, v, shift_k, ssm_k, ssm_D):
        B, S, D = q.shape
        ks = shift_k.shape[-1]
        k_pad = jnp.pad(k, ((0, 0), (ks - 1, 0), (0, 0)))
        k_shift = jnp.zeros_like(k)
        for t in range(ks):
            k_shift = k_shift + k_pad[:, t:t + S, :] * shift_k[:, ks - 1 - t][None, None, :]
        kv = k_shift * v
        L = 2 * S
        kv_pad = jnp.pad(kv, ((0, 0), (0, S), (0, 0)))
        kf_pad = jnp.pad(ssm_k, ((0, 0), (0, S)))
        kv_f = (lambda x, axes=(-2,-1): jnp.fft.rfft2(x.astype(jnp.float32), axes=axes))(kv_pad[:, None, :, :], axes=(1, 2))
        kf_f = (lambda x, axes=(-2,-1): jnp.fft.rfft2(x.astype(jnp.float32), axes=axes))(kf_pad[:, None, :], axes=(1, 2))
        kf_f = (lambda x, *d: x.transpose(*d))(kf_f, 1, 2, 0)
        y_f = kv_f * kf_f[None, :, :, :]
        y = (lambda x, s, axes=(-2,-1): jnp.fft.irfft2(x, s=s, axes=axes).astype(jnp.bfloat16))(y_f, (1, L), axes=(1, 2))[:, 0, :S, :]
        y = y + kv * ssm_D[None, None, :]
        return q * y

    def _B_ref(q, k, v, shift_k, ssm_k, ssm_D):
        B, S, D = q.shape
        ks = shift_k.shape[-1]
        k_pad = jnp.pad(k, ((0, 0), (ks - 1, 0), (0, 0)))
        k_shift = jnp.zeros_like(k)
        for t in range(ks):
            k_shift = k_shift + k_pad[:, t:t + S, :] * shift_k[:, ks - 1 - t][None, None, :]
        kv = k_shift * v
        L = 2 * S
        kv_pad = jnp.pad(kv, ((0, 0), (0, S), (0, 0)))
        kf_pad = jnp.pad(ssm_k, ((0, 0), (0, S)))
        kv_f = (lambda x, axes=(-2,-1): jnp.fft.rfft2(x.astype(jnp.float32), axes=axes))(kv_pad[:, None, :, :], axes=(1, 2))
        kf_f = (lambda x, axes=(-2,-1): jnp.fft.rfft2(x.astype(jnp.float32), axes=axes))(kf_pad[:, None, :], axes=(1, 2))
        kf_f = (lambda x, *d: x.transpose(*d))(kf_f, 1, 2, 0)
        y_f = kv_f * kf_f[None, :, :, :]
        y = (lambda x, s, axes=(-2,-1): jnp.fft.irfft2(x, s=s, axes=axes).astype(jnp.bfloat16))(y_f, (1, L), axes=(1, 2))[:, 0, :S, :]
        y = y + kv * ssm_D[None, None, :]
        return q * y

    x = A_q
    g = _sigmoid((x * gate_w).sum(-1, keepdims=True))
    a = _A_ref(x, A_k, A_v, A_shift_k, A_ssm_k, A_ssm_D)
    b = _B_ref(x, B_k, B_v, B_shift_k, B_ssm_k, B_ssm_D)
    return g * a + (1 - g) * b
```

```python
import jax
import jax.numpy as jnp
import numpy as np
from jax import lax
from jax.experimental import pallas as pl
from jax.experimental.pallas import tpu as pltpu

S = 2048
D = 640
CT = 128
NT = D // CT
M = 128
NTAU = S // M
PS = 264
ZS = 272
KPAD = 16

bf16 = jnp.bfloat16
f32 = jnp.float32
u32 = jnp.uint32


def _bf16_bits(a):
    u = np.ascontiguousarray(a, dtype=np.float32).view(np.uint32).astype(np.uint64)
    r = (u + 0x7FFF + ((u >> 16) & 1)) >> 16
    return r.astype(np.uint32)


def _pack_rows(a):
    b = _bf16_bits(a)
    return (b[0::2] | (b[1::2] << 16)).astype(np.uint32)


def make_tables(R):
    kap = 2 * np.arange(M)
    om = np.pi * (2 * kap + 1) / (256.0 * R)
    m = np.arange(M)
    FX, G = [], []
    for r in range(R):
        ph = np.outer(om, R * m + r)
        F = np.stack([np.cos(ph).reshape(16, 8, M), -np.sin(ph).reshape(16, 8, M)], 1).reshape(2 * M, M)
        FX.append(_pack_rows(F))
        Gm = np.empty((M, 16, 2, 8))
        Gm[:, :, 0, :] = (np.cos(ph).T / (128.0 * R)).reshape(M, 16, 8)
        Gm[:, :, 1, :] = (-np.sin(ph).T / (128.0 * R)).reshape(M, 16, 8)
        G.append(_pack_rows(Gm.reshape(M, 2 * M)))
    return np.stack(FX), np.stack(G)


def mof(x, n):
    return x if isinstance(x, int) else pl.multiple_of(x, n)


def lo(w):
    return pltpu.bitcast(w << 16, f32)


def hi(w):
    return pltpu.bitcast(w & jnp.uint32(0xFFFF0000), f32)


_ORDERS = ["fmipt", "tfmip", "ftmip", "fmtip", "fmitp", "tfimp", "ftimp", "fitmp", "tifmp", "ftpmi", "tfpmi", "fptmi", "fmpti", "ftmpi"]


def _build(R=4, dma=1, order="m0.i0.m1.m3.e.m2.i2.i1.i3", gauss=0, park=1, unroll=0, gu=4,
          o_fm="x.h.m.p.t", o_a="h0.h1.h2.h3.m0.m1.m2.x0.x1.x2.x3.p0.p1.p2.m3.i3.p3.i0.e.i1.i2.t3.t0.t1.t2", o_b="h.m.x.p.i.t"):
    NB = NTAU // R
    WS = R // 2
    WPB = 64 * R
    FXt, Gt = make_tables(R)

    wt, pk = u32, 2

    def words(ref, idx, start, n, stride=1):
        sl = pl.ds(start, n) if stride == 1 else pl.ds(start, n, stride=stride)
        r_ = ref if ref.dtype == u32 else ref.bitcast(u32)
        return r_[(*idx, sl, slice(None))]

    def kernel(q_h, kA_h, vA_h, hA_h, kB_h, vB_h, hB_h,
               skA_h, skB_h, dA_h, dB_h, gw_h,
               FX_h, G_h,
               out_h,
               skA_ref, skB_ref, dA_ref, dB_ref, gw_ref, FX_ref, G_ref,
               qb, kb, vb, hb, ob,
               PB, GW, KV, HT, TXA, THA, TXB, THB, ZA, ZB, YA, YB, ON, GT, MT,
               sem_in, sem_first, sem_out, sem_small):

        def hview(src):
            return src.bitcast(u32)

        RB = R * M

        def in_copy(kind, t, blk=None):
            src_ = {"q": q_h, "kA": kA_h, "vA": vA_h, "kB": kB_h, "vB": vB_h, "hA": hA_h, "hB": hB_h}[kind]
            slot = ["q", "kA", "vA", "hA", "kB", "vB", "hB"].index(kind)
            u = 2 * t + int(kind[-1] == "B")
            sem = sem_in.at[slot, t] if blk is None else sem_first.at[slot, t * NB + blk]
            r0, nr = (0, S) if blk is None else (blk * RB, RB)
            if kind[0] == "h":
                s, d = src_.at[pl.ds(t * CT, CT), pl.ds(r0, nr)], hb.at[u, :, pl.ds(r0, nr)]
            else:
                s = hview(src_).at[pl.ds(r0 // pk, nr // pk), pl.ds(t * CT, CT)]
                off = KPAD if kind[0] == "k" else 0
                dst = {"q": qb.at[t], "k": kb.at[u], "v": vb.at[u]}[kind[0]]
                d = dst.at[pl.ds((off + r0) // pk, nr // pk), :]
            return pltpu.make_async_copy(s, d, sem)

        def out_copy(t, blk):
            rows = pl.ds(blk * RB, RB)
            return pltpu.make_async_copy(ob.at[t, rows, :], out_h.at[rows, pl.ds(t * CT, CT)], sem_out.at[t, blk])

        def blocks(br, t, blks, op):
            for blk in blks:
                for n in ("h", "k", "v"):
                    cp_ = in_copy(n + br, t, blk)
                    cp_.start() if op == "start" else cp_.wait()

        def wait_unit(br, t):
            for n in ("h", "k", "v"):
                in_copy(n + br, t).wait()

        first = [(n + "A", 0, blk) for blk in range(NB) for n in ("h", "k", "v")]
        small = [pltpu.make_async_copy(s_, d_, sem_small.at[i_]) for i_, (s_, d_) in enumerate(
            [(skA_h, skA_ref), (skB_h, skB_ref), (dA_h, dA_ref), (dB_h, dB_ref), (gw_h, gw_ref),
             (FX_h, FX_ref), (G_h, G_ref)])]
        for cp in small[:6]:
            cp.start()
        for piece in first[:6]:
            in_copy(*piece).start()
        for cp in small[:5]:
            cp.wait()

        skA = skA_ref[...].astype(f32)
        skB = skB_ref[...].astype(f32)
        dA = dA_ref[...].astype(f32)
        dB = dB_ref[...].astype(f32)
        gw = gw_ref[...].astype(f32)
        for t in range(NT):
            sl = slice(t * CT, (t + 1) * CT)
            for u, sk, dd in ((2 * t, skA, dA), (2 * t + 1, skB, dB)):
                for j in range(4):
                    PB[u, j] = jnp.broadcast_to(sk[j:j + 1, sl], (8, CT))
                PB[u, 4] = jnp.broadcast_to(dd[sl].reshape(1, CT), (8, CT))
                kb[u, 0:KPAD // pk, :] = jnp.zeros((KPAD // pk, CT), wt)
            GW[t] = jnp.broadcast_to(gw[sl].reshape(1, CT), (8, CT))
        kpw = KPAD // 2
        NU = 2 * NT
        YA[NT] = jnp.zeros((S, CT), f32)
        YB[NT] = jnp.zeros((S, CT), f32)
        qb[NT] = jnp.zeros(qb.shape[1:], wt)
        GT[...] = jnp.zeros(GT.shape, f32)

        def bcast(x, n):
            return jnp.broadcast_to(x[None], (n // 8, 8, CT)).reshape(n, CT)

        HO = 16

        def st_tile(T, tau, y, off=0):
            r0 = mof(tau * 16, 16)
            for p in range(16):
                T[pl.ds(off + p * PS + r0, 16), :] = y[p * 16:(p + 1) * 16, :]

        def prep_h(t, b, slot, cs=range(R)):
            for c in cs:
                l0 = mof((b * R + c) * M, M)
                HT[slot, c * 64:(c + 1) * 64, :] = pltpu.bitcast(hb[t, :, pl.ds(l0, M)].T, u32)

        def prep(t, b, slot, rs=range(R), cache=None):
            cache = {} if cache is None else cache
            base = b * WPB
            if "w" not in cache:
                cache["w"] = [bcast(PB[t, j], M) for j in range(4)]
            w = cache["w"]

            def kres(s):
                if s not in cache:
                    wr, hf = s >> 1, s & 1
                    key = ("w", wr)
                    if key not in cache:
                        cache[key] = words(kb, (t,), base + kpw + wr, M, WS)
                    cache[s] = hi(cache[key]) if hf else lo(cache[key])
                return cache[s]

            for r in rs:
                acc = kres(r) * w[0]
                for j in range(1, 4):
                    acc = acc + kres(r - j) * w[j]
                if ("v", r >> 1) not in cache:
                    cache[("v", r >> 1)] = words(vb, (t,), base + (r >> 1), M, WS)
                vw = cache[("v", r >> 1)]
                v = hi(vw) if r & 1 else lo(vw)
                KV[slot, r * M:(r + 1) * M, :] = (acc * v).astype(bf16)

        def fwd_x(br, b, slot, rs=range(R)):
            TX = TXA if br == "A" else TXB
            for r in rs:
                kv = pltpu.bitcast(words(KV, (slot,), r * 64, 64), bf16)
                F = pltpu.bitcast(FX_ref[r], bf16)
                st_tile(TX, b * R + r, jnp.dot(F, kv, preferred_element_type=f32))

        def fwd_h(br, b, slot, rs=range(R), cache=None):
            cache = {} if cache is None else cache
            TH = THA if br == "A" else THB
            for r in rs:
                c = r >> 1
                if c not in cache:
                    cache[c] = (HT[slot, pl.ds(c, 64, stride=2 * WS), :], HT[slot, pl.ds(c + WS, 64, stride=2 * WS), :])
                A, B = cache[c]
                if r & 1 == 0:
                    hw = (A & jnp.uint32(0xFFFF)) | (B << 16)
                else:
                    hw = (A >> 16) | (B & jnp.uint32(0xFFFF0000))
                F = pltpu.bitcast(FX_ref[r], bf16)
                st_tile(TH, b * R + r, jnp.dot(F, pltpu.bitcast(hw, bf16), preferred_element_type=f32), HO)

        def mac(br, t, b, pps=range(R)):
            TX, TH = (TXA, THA) if br == "A" else (TXB, THB)
            Z = ZA if br == "A" else ZB
            dvec = PB[2 * t + (br == "B"), 4]
            for pp in pps:
                prow0 = mof((b * R + pp) * PS, 8)
                zrow0 = mof((b * R + pp) * ZS, 16)

                def ld(T, tau):
                    off = HO if T is TH else 0
                    return (T[pl.ds(off + prow0 + tau * 16, 8), :], T[pl.ds(off + prow0 + tau * 16 + 8, 8), :])

                def group(Xg, Hg):
                    Y = [None] * NB
                    if gauss:
                        xs = [Xg[j][0] + Xg[j][1] for j in range(NB)]
                    for m_ in range(NB):
                        hr, hi = Hg[m_]
                        if m_ == 0:
                            hr = hr + dvec
                        else:
                            hr, hi = hr - Hg[m_ - 1][1], hi + Hg[m_ - 1][0]
                        if gauss:
                            hd, he = hi - hr, hr + hi
                        for j in range(NB - m_):
                            xr, xi = Xg[j]
                            i = j + m_
                            if gauss:
                                c3 = (hr * xs[j], hd * xr, he * xi)
                                Y[i] = c3 if Y[i] is None else tuple(u + v for u, v in zip(Y[i], c3))
                            elif Y[i] is None:
                                Y[i] = (xr * hr - xi * hi, xr * hi + xi * hr)
                            else:
                                Y[i] = (Y[i][0] + xr * hr - xi * hi, Y[i][1] + xr * hi + xi * hr)
                    if gauss:
                        Y = [(y[0] - y[2], y[0] + y[1]) for y in Y]
                    return Y

                def stz(tau, zr, zi):
                    Z[pl.ds(zrow0 + tau * 16, 16), :] = jnp.concatenate([zr, zi], axis=0).astype(bf16)

                if R == 2:
                    Ys = []
                    for rp in range(2):
                        sg = (lambda u, v: u + v) if rp == 0 else (lambda u, v: u - v)

                        def bf2(T, j):
                            (a0, a1), (c0, c1) = ld(T, 2 * j), ld(T, 2 * j + 1)
                            return (sg(a0, c0), sg(a1, c1))
                        Ys.append(group([bf2(TX, j) for j in range(NB)], [bf2(TH, j) for j in range(NB)]))
                        if rp == 0 and park:
                            for i in range(NB):
                                MT[pp, 2 * i] = Ys[0][i][0]
                                MT[pp, 2 * i + 1] = Ys[0][i][1]
                    for i in range(NB):
                        a0, a1 = (MT[pp, 2 * i], MT[pp, 2 * i + 1]) if park else Ys[0][i]
                        c0, c1 = Ys[1][i]
                        stz(2 * i, a0 + c0, a1 + c1)
                        stz(2 * i + 1, a0 - c0, a1 - c1)
                else:
                    def pairA(T, j):
                        (r0, i0), (r1, i1), (r2, i2), (r3, i3) = [ld(T, 4 * j + r) for r in range(4)]
                        ar, ai, cr, ci = r0 + r2, i0 + i2, r1 + r3, i1 + i3
                        return [(ar + cr, ai + ci), (ar - cr, ai - ci)]

                    def pairB(T, j):
                        (r0, i0), (r1, i1), (r2, i2), (r3, i3) = [ld(T, 4 * j + r) for r in range(4)]
                        br_, bi, dr, di = r0 - r2, i0 - i2, r1 - r3, i1 - i3
                        return [(br_ + di, bi - dr), (br_ - di, bi + dr)]

                    def pair_mac(pair, emit):
                        X = [pair(TX, j) for j in range(NB)]
                        Y = [[None] * NB for _ in range(2)]
                        prev = None
                        for m_ in range(NB):
                            raw = pair(TH, m_)
                            for g in range(2):
                                hr, hi = raw[g]
                                if m_ == 0:
                                    hr = hr + dvec
                                else:
                                    hr, hi = hr - prev[g][1], hi + prev[g][0]
                                for j in range(NB - m_):
                                    xr, xi = X[j][g]
                                    i = j + m_
                                    if Y[g][i] is None:
                                        Y[g][i] = (xr * hr - xi * hi, xr * hi + xi * hr)
                                    else:
                                        Y[g][i] = (Y[g][i][0] + (xr * hr - xi * hi), Y[g][i][1] + (xr * hi + xi * hr))
                            prev = raw
                            emit(m_, Y[0][m_], Y[1][m_])

                    SD = [None] * NB

                    def emitA(i, y0, y2):
                        sd = (y0[0] + y2[0], y0[1] + y2[1], y0[0] - y2[0], y0[1] - y2[1])
                        if park:
                            for c in range(4):
                                MT[pp, 4 * i + c] = sd[c]
                        else:
                            SD[i] = sd

                    def emitB(i, y1, y3):
                        sr, si, dr, di = [MT[pp, 4 * i + c] for c in range(4)] if park else SD[i]
                        ur, ui = y1[0] + y3[0], y1[1] + y3[1]
                        vr, vi = y1[0] - y3[0], y1[1] - y3[1]
                        stz(4 * i + 0, sr + ur, si + ui)
                        stz(4 * i + 2, sr - ur, si - ui)
                        stz(4 * i + 1, dr - vi, di + vr)
                        stz(4 * i + 3, dr + vi, di - vr)

                    pair_mac(pairA, emitA)
                    pair_mac(pairB, emitB)

        def inv(br, t, b, rs=range(R), cache=None, fin=True):
            cache = {} if cache is None else cache
            Z = ZA if br == "A" else ZB
            for r in rs:
                tau = b * R + r
                zw = jnp.concatenate(
                    [words(Z, (), mof(p * (ZS // 2) + tau * 8, 8), 8) for p in range(16)], axis=0)
                Gm = pltpu.bitcast(G_ref[r], bf16)
                y = jnp.dot(Gm, pltpu.bitcast(zw, bf16), preferred_element_type=f32)
                y0 = mof(tau * M, M)
                (YA if br == "A" else YB)[t, pl.ds(y0, M), :] = y

        def epi(t, b, rs=range(R), cache=None, fin=True, slot=0):
            cache = {} if cache is None else cache
            for r in rs:
                y0 = mof((b * R + r) * M, M)
                if (r >> 1) not in cache:
                    cache[r >> 1] = words(qb, (t,), b * WPB + (r >> 1), M, WS)
                qwd = cache[r >> 1]
                qv = hi(qwd) if r & 1 else lo(qwd)
                g = GT[r & 1, pl.ds(b * WPB + (r >> 1), M, stride=WS), :]
                yb = YB[t, pl.ds(y0, M), :]
                ON[slot, pl.ds(r, M, stride=R), :] = qv * (yb + g * (YA[t, pl.ds(y0, M), :] - yb))
            if fin:
                ob[t, pl.ds(mof(b * R * M, M), R * M), :] = ON[slot].astype(bf16)

        def gate(c):
            r0 = mof(c * M, M)
            accs = [None, None]
            for t in range(NT):
                wd = words(qb, (t,), r0, M)
                wv = bcast(GW[t], M)
                for hf in range(2):
                    x = (hi(wd) if hf else lo(wd)) * wv
                    accs[hf] = x if accs[hf] is None else accs[hf] + x
            for hf in range(2):
                s = jnp.sum(accs[hf], axis=1, keepdims=True)
                GT[hf, pl.ds(r0, M), :] = jnp.broadcast_to(0.5 * jnp.tanh(0.5 * s) + 0.5, (M, CT))

        def scoped(name, fn):
            del name
            fn()

        def loop(n, fn, unr=False):
            if unr:
                for b in range(n):
                    fn(b)
                return

            def body(b, carry):
                fn(b)
                return carry
            lax.fori_loop(0, n, body, 0)

        def phase(fw, mc, iv, mid=None, order=order, static=False, ep=None):
            def body(b, par=None):
                if par is None:
                    par = b % 2 if isinstance(b, int) else lax.rem(b, 2)
                def do_prep(fn):
                    u = 2 * fw[1] + (fw[0] == "B")
                    if isinstance(b, int):
                        un, bn = u + (b + 1) // NB, (b + 1) % NB
                    else:
                        un, bn = u + lax.div(b + 1, NB), lax.rem(b + 1, NB)
                    un = min(un, NU - 1) if isinstance(un, int) else jnp.minimum(un, NU - 1)
                    fn(un, bn, 1 - par)
                caches = {"p": {}, "h": {}, "i": {}}
                toks = []
                for key in order.split("."):
                    if len(key) == 1:
                        toks += [(key, list(range(R)))]
                    else:
                        toks.append((key[0], ["0123abcd".index(c_) % 4 for c_ in key[1:]]))
                for kind, idx in toks:
                    if kind == "x" and fw:
                        fwd_x(fw[0], b, par, idx)
                    elif kind == "h" and fw:
                        fwd_h(fw[0], b, par, idx, caches["h"])
                    elif kind == "m" and mc:
                        mac(*mc, b, idx)
                    elif kind == "i" and iv:
                        inv(*iv, b, idx, caches["i"], fin=False)
                    elif kind == "e" and ep is not None:
                        epi(ep, b)
                    elif kind == "p" and fw:
                        do_prep(lambda un, bn, sl: prep(un, bn, sl, idx, caches["p"]))
                    elif kind == "t" and fw:
                        do_prep(lambda un, bn, sl: prep_h(un, bn, sl, idx))
            if static:
                for b in range(NB):
                    if mid and b == NB - 1:
                        mid()
                    body(b)
            elif mid:
                lax.fori_loop(0, NB // 2, lambda b, c: (body(b), c)[1], 0)
                mid()
                lax.fori_loop(NB // 2, NB, lambda b, c: (body(b), c)[1], 0)
            else:
                loop(NB, body)

        def start_unit(br, t):
            for n in ("h", "k", "v"):
                in_copy(n + br, t).start()

        for piece in first[:3]:
            in_copy(*piece).wait()
        for piece in first[6:12]:
            in_copy(*piece).start()
        small[5].wait()
        scoped("prep0", lambda: (prep_h(0, 0, 0), prep(0, 0, 0)))
        if True:
            for b in range(NB):
                if b + 1 < NB:
                    for piece in first[3 * (b + 1):3 * (b + 2)]:
                        in_copy(*piece).wait()
                    if b == 0:
                        for n in ("h", "k", "v"):
                            in_copy(n + "B", 0, 0).start()
                    if b == 1:
                        for blk in range(1, NB):
                            for n in ("h", "k", "v"):
                                in_copy(n + "B", 0, blk).start()
                else:
                    for n in ("h", "k", "v"):
                        in_copy(n + "B", 0, 0).wait()
                    small[6].start()
                    blocks("A", 1, (0, 1), "start")
                fwd_h("A", b, b % 2)
                fwd_x("A", b, b % 2)
                un, bn = (b + 1) // NB, (b + 1) % NB
                prep(un, bn, (b + 1) % 2)
                prep_h(un, bn, (b + 1) % 2)

        def mid_fm():
            blocks("B", 0, (NB - 1,), "wait")
            scoped("w2", lambda: blocks("A", 1, (0,), "wait"))
            scoped("wG", lambda: small[6].wait())
            start_unit("B", 1)

        if True:
            blocks("B", 0, (1, 2), "wait")
        blocks("A", 1, (2, 3), "start")
        scoped("P_fm", lambda: phase(("B", 0), ("A", 0), None, mid=mid_fm, order=o_fm))

        def tile_body(t, carry):
            more = t + 2 < NT

            def mid_b():
                @pl.when(t == 0)
                def _():
                    blocks("A", 1, (NB - 1,), "wait")
                scoped("wB", lambda: wait_unit("B", t + 1))

                @pl.when(t == 0)
                def _():
                    start_unit("B", 2)

                @pl.when(t == 1)
                def _():
                    start_unit("A", 3)

                @pl.when(t == 2)
                def _():
                    start_unit("B", 4)

                @pl.when(t == NT - 2)
                def _():
                    for tt in range(2):
                        for blk in range(NB):
                            out_copy(tt, blk).start()

            def mid_a():
                @pl.when(more)
                def _():
                    scoped("wA", lambda: wait_unit("A", t + 2))

                @pl.when(t == 0)
                def _():
                    for tt in range(NT):
                        in_copy("q", tt).start()

                @pl.when(t == 1)
                def _():
                    start_unit("A", 4)

            @pl.when(t == 0)
            def _():
                scoped("w3", lambda: blocks("A", 1, (1, 2), "wait"))
                start_unit("A", 2)
            scoped("P_B", lambda: phase(("A", t + 1), ("B", t), ("A", t), mid=mid_b, order=o_b))

            @pl.when(t == 1)
            def _():
                if True:
                    for tt in range(NT):
                        in_copy("q", tt).wait()
                start_unit("B", 3)
                scoped("gate", lambda: loop(S // (2 * M) // gu, lambda c: [gate(c * gu + i_) for i_ in range(gu)]))

            ep = jnp.where(t == 0, NT, t - 1)
            scoped("P_A", lambda: phase(("B", t + 1), ("A", t + 1), ("B", t), mid=mid_a, order=o_a, ep=ep))
            return carry

        lax.fori_loop(0, NT - 1, tile_body, 0)
        tl = NT - 1
        for blk in range(NB):
            out_copy(2, blk).start()
        def mid_mi():
            for blk in range(NB // 2):
                out_copy(tl - 1, blk).start()

        scoped("P_mi", lambda: phase(None, ("B", tl), ("A", tl), mid=mid_mi, ep=tl - 1))
        for blk in range(NB // 2, NB):
            out_copy(tl - 1, blk).start()
        if True:
            for b in range(NB):
                inv("B", tl, b)
                if b > 0:
                    epi(tl, b - 1, slot=b % 2)
                    out_copy(tl, b - 1).start()
            epi(tl, NB - 1, slot=NB % 2)
            out_copy(tl, NB - 1).start()
        if True:
            for t in range(NT):
                for blk in range(NB):
                    out_copy(t, blk).wait()

    hbm = pl.BlockSpec(memory_space=pl.ANY)
    vmem = pl.BlockSpec(memory_space=pltpu.VMEM)

    @jax.jit
    def fn(A_q, A_k, A_v, A_shift_k, A_ssm_k, A_ssm_D, B_q, B_k, B_v, B_shift_k, B_ssm_k, B_ssm_D, gate_w):
        del B_q
        out = pl.pallas_call(
            kernel,
            out_shape=jax.ShapeDtypeStruct((S, D), bf16),
            in_specs=[hbm] * 14,
            out_specs=hbm,
            scratch_shapes=[
                pltpu.VMEM((4, D), bf16), pltpu.VMEM((4, D), bf16),
                pltpu.VMEM((D,), bf16), pltpu.VMEM((D,), bf16), pltpu.VMEM((D,), bf16),
                pltpu.VMEM(FXt.shape, u32), pltpu.VMEM(Gt.shape, u32),
                pltpu.VMEM((NT + 1, S // pk, CT), wt),
                pltpu.VMEM((2 * NT, (KPAD + S) // pk, CT), wt),
                pltpu.VMEM((2 * NT, S // pk, CT), wt),
                pltpu.VMEM((2 * NT, CT, S), bf16),
                pltpu.VMEM((NT + 1, S, CT), bf16),
                pltpu.VMEM((2 * NT, 5, 8, CT), f32),
                pltpu.VMEM((NT, 8, CT), f32),
                pltpu.VMEM((2, R * M, CT), bf16),
                pltpu.VMEM((2, 64 * R, CT), u32),
                pltpu.VMEM((16 * PS + 16, CT), f32),
                pltpu.VMEM((16 * PS + 16, CT), f32),
                pltpu.VMEM((16 * PS + 16, CT), f32),
                pltpu.VMEM((16 * PS + 16, CT), f32),
                pltpu.VMEM((16 * ZS, CT), bf16),
                pltpu.VMEM((16 * ZS, CT), bf16),
                pltpu.VMEM((NT + 1, S, CT), f32),
                pltpu.VMEM((NT + 1, S, CT), f32),
                pltpu.VMEM((2, R * M, CT), f32),
                pltpu.VMEM((2, S // 2, CT), f32),
                pltpu.VMEM((R, 16, 8, CT), f32),
                pltpu.SemaphoreType.DMA((7, NT)),
                pltpu.SemaphoreType.DMA((7, 2 * NB)),
                pltpu.SemaphoreType.DMA((NT, NB)),
                pltpu.SemaphoreType.DMA((8,)),
            ],
            compiler_params=pltpu.CompilerParams(vmem_limit_bytes=100 * 1024 * 1024),
            name="h3mix",
        )(A_q.reshape(S, D), A_k.reshape(S, D), A_v.reshape(S, D), A_ssm_k,
          B_k.reshape(S, D), B_v.reshape(S, D), B_ssm_k,
          A_shift_k.T, B_shift_k.T, A_ssm_D, B_ssm_D, gate_w,
          FXt, Gt)
        return out.reshape(1, S, D)

    return fn


pallas_gated_mix__ssm_conv_h3__ssm_conv_h3__prompt_kernel = _build()
```

```python
import jax
import jax.numpy as jnp
import numpy as np
from jax import lax
from jax.experimental import pallas as pl
from jax.experimental.pallas import tpu as pltpu

S = 2048
D = 640
CT = 128
NT = D // CT
M = 128
NTAU = S // M
PS = 264
ZS = 272
KPAD = 16

bf16 = jnp.bfloat16
f32 = jnp.float32
u32 = jnp.uint32


def _bf16_bits(a):
    u = np.ascontiguousarray(a, dtype=np.float32).view(np.uint32).astype(np.uint64)
    r = (u + 0x7FFF + ((u >> 16) & 1)) >> 16
    return r.astype(np.uint32)


def _pack_rows(a):
    b = _bf16_bits(a)
    return (b[0::2] | (b[1::2] << 16)).astype(np.uint32)


def make_tables(R):
    kap = 2 * np.arange(M)
    om = np.pi * (2 * kap + 1) / (256.0 * R)
    m = np.arange(M)
    FX, G = [], []
    for r in range(R):
        ph = np.outer(om, R * m + r)
        F = np.stack([np.cos(ph).reshape(16, 8, M), -np.sin(ph).reshape(16, 8, M)], 1).reshape(2 * M, M)
        FX.append(_pack_rows(F))
        Gm = np.empty((M, 16, 2, 8))
        Gm[:, :, 0, :] = (np.cos(ph).T / (128.0 * R)).reshape(M, 16, 8)
        Gm[:, :, 1, :] = (-np.sin(ph).T / (128.0 * R)).reshape(M, 16, 8)
        G.append(_pack_rows(Gm.reshape(M, 2 * M)))
    return np.stack(FX), np.stack(G)


def mof(x, n):
    return x if isinstance(x, int) else pl.multiple_of(x, n)


def lo(w):
    return pltpu.bitcast(w << 16, f32)


def hi(w):
    return pltpu.bitcast(w & jnp.uint32(0xFFFF0000), f32)


_ORDERS = ["fmipt", "tfmip", "ftmip", "fmtip", "fmitp", "tfimp", "ftimp", "fitmp", "tifmp", "ftpmi", "tfpmi", "fptmi", "fmpti", "ftmpi"]


def _build(R=4, dma=1, order="m0.i0.m1.m3.e.m2.i2.i1.i3", gauss=0, park=1, unroll=0, gu=4,
          o_fm="x.h.m.p.t", o_a="h0.h1.h2.h3.m0.m1.m2.x0.x1.x2.x3.p0.p1.p2.m3.i3.p3.i0.e.i1.i2.t3.t0.t1.t2", o_b="h.m.x.p.i.t"):
    NB = NTAU // R
    WS = R // 2
    WPB = 64 * R
    FXt, Gt = make_tables(R)

    wt, pk = u32, 2

    def words(ref, idx, start, n, stride=1):
        sl = pl.ds(start, n) if stride == 1 else pl.ds(start, n, stride=stride)
        r_ = ref if ref.dtype == u32 else ref.bitcast(u32)
        return r_[(*idx, sl, slice(None))]

    def kernel(q_h, kA_h, vA_h, hA_h, kB_h, vB_h, hB_h,
               skA_h, skB_h, dA_h, dB_h, gw_h,
               FX_h, G_h,
               out_h,
               skA_ref, skB_ref, dA_ref, dB_ref, gw_ref, FX_ref, G_ref,
               qb, kb, vb, hb, ob,
               PB, GW, KV, HT, TXA, THA, TXB, THB, ZA, ZB, YA, YB, ON, GT, MT,
               sem_in, sem_first, sem_out, sem_small):

        def hview(src):
            return src.bitcast(u32)

        RB = R * M

        def in_copy(kind, t, blk=None):
            src_ = {"q": q_h, "kA": kA_h, "vA": vA_h, "kB": kB_h, "vB": vB_h, "hA": hA_h, "hB": hB_h}[kind]
            slot = ["q", "kA", "vA", "hA", "kB", "vB", "hB"].index(kind)
            u = 2 * t + int(kind[-1] == "B")
            sem = sem_in.at[slot, t] if blk is None else sem_first.at[slot, t * NB + blk]
            r0, nr = (0, S) if blk is None else (blk * RB, RB)
            if kind[0] == "h":
                s, d = src_.at[pl.ds(t * CT, CT), pl.ds(r0, nr)], hb.at[u, :, pl.ds(r0, nr)]
            else:
                s = hview(src_).at[pl.ds(r0 // pk, nr // pk), pl.ds(t * CT, CT)]
                off = KPAD if kind[0] == "k" else 0
                dst = {"q": qb.at[t], "k": kb.at[u], "v": vb.at[u]}[kind[0]]
                d = dst.at[pl.ds((off + r0) // pk, nr // pk), :]
            return pltpu.make_async_copy(s, d, sem)

        def out_copy(t, blk):
            rows = pl.ds(blk * RB, RB)
            return pltpu.make_async_copy(ob.at[t, rows, :], out_h.at[rows, pl.ds(t * CT, CT)], sem_out.at[t, blk])

        def blocks(br, t, blks, op):
            for blk in blks:
                for n in ("h", "k", "v"):
                    cp_ = in_copy(n + br, t, blk)
                    cp_.start() if op == "start" else cp_.wait()

        def wait_unit(br, t):
            for n in ("h", "k", "v"):
                in_copy(n + br, t).wait()

        first = [(n + "A", 0, blk) for blk in range(NB) for n in ("h", "k", "v")]
        small = [pltpu.make_async_copy(s_, d_, sem_small.at[i_]) for i_, (s_, d_) in enumerate(
            [(skA_h, skA_ref), (skB_h, skB_ref), (dA_h, dA_ref), (dB_h, dB_ref), (gw_h, gw_ref),
             (FX_h, FX_ref), (G_h, G_ref)])]
        for cp in small[:6]:
            cp.start()
        for piece in first[:6]:
            in_copy(*piece).start()
        YA[NT] = jnp.zeros((S, CT), f32)
        YB[NT] = jnp.zeros((S, CT), f32)
        qb[NT] = jnp.zeros(qb.shape[1:], wt)
        GT[...] = jnp.zeros(GT.shape, f32)
        if True:
            for cp in small[:5]:
                cp.wait()

        skA = skA_ref[...].astype(f32)
        skB = skB_ref[...].astype(f32)
        dA = dA_ref[...].astype(f32)
        dB = dB_ref[...].astype(f32)
        gw = gw_ref[...].astype(f32)
        for t in range(NT):
            sl = slice(t * CT, (t + 1) * CT)
            for u, sk, dd in ((2 * t, skA, dA), (2 * t + 1, skB, dB)):
                for j in range(4):
                    PB[u, j] = jnp.broadcast_to(sk[j:j + 1, sl], (8, CT))
                PB[u, 4] = jnp.broadcast_to(dd[sl].reshape(1, CT), (8, CT))
                kb[u, 0:KPAD // pk, :] = jnp.zeros((KPAD // pk, CT), wt)
            GW[t] = jnp.broadcast_to(gw[sl].reshape(1, CT), (8, CT))
        kpw = KPAD // 2
        NU = 2 * NT
        def bcast(x, n):
            return jnp.broadcast_to(x[None], (n // 8, 8, CT)).reshape(n, CT)

        HO = 16

        def st_tile(T, tau, y, off=0):
            r0 = mof(tau * 16, 16)
            for p in range(16):
                T[pl.ds(off + p * PS + r0, 16), :] = y[p * 16:(p + 1) * 16, :]

        def prep_h(t, b, slot, cs=range(R)):
            for c in cs:
                l0 = mof((b * R + c) * M, M)
                HT[slot, c * 64:(c + 1) * 64, :] = pltpu.bitcast(hb[t, :, pl.ds(l0, M)].T, u32)

        def prep(t, b, slot, rs=range(R), cache=None):
            cache = {} if cache is None else cache
            base = b * WPB
            if "w" not in cache:
                cache["w"] = [bcast(PB[t, j], M) for j in range(4)]
            w = cache["w"]

            def kres(s):
                if s not in cache:
                    wr, hf = s >> 1, s & 1
                    key = ("w", wr)
                    if key not in cache:
                        cache[key] = words(kb, (t,), base + kpw + wr, M, WS)
                    cache[s] = hi(cache[key]) if hf else lo(cache[key])
                return cache[s]

            for r in rs:
                acc = kres(r) * w[0]
                for j in range(1, 4):
                    acc = acc + kres(r - j) * w[j]
                if ("v", r >> 1) not in cache:
                    cache[("v", r >> 1)] = words(vb, (t,), base + (r >> 1), M, WS)
                vw = cache[("v", r >> 1)]
                v = hi(vw) if r & 1 else lo(vw)
                KV[slot, r * M:(r + 1) * M, :] = (acc * v).astype(bf16)

        def fwd_x(br, b, slot, rs=range(R)):
            TX = TXA if br == "A" else TXB
            for r in rs:
                kv = pltpu.bitcast(words(KV, (slot,), r * 64, 64), bf16)
                F = pltpu.bitcast(FX_ref[r], bf16)
                st_tile(TX, b * R + r, jnp.dot(F, kv, preferred_element_type=f32))

        def fwd_h(br, b, slot, rs=range(R), cache=None):
            cache = {} if cache is None else cache
            TH = THA if br == "A" else THB
            for r in rs:
                c = r >> 1
                if c not in cache:
                    cache[c] = (HT[slot, pl.ds(c, 64, stride=2 * WS), :], HT[slot, pl.ds(c + WS, 64, stride=2 * WS), :])
                A, B = cache[c]
                if r & 1 == 0:
                    hw = (A & jnp.uint32(0xFFFF)) | (B << 16)
                else:
                    hw = (A >> 16) | (B & jnp.uint32(0xFFFF0000))
                F = pltpu.bitcast(FX_ref[r], bf16)
                st_tile(TH, b * R + r, jnp.dot(F, pltpu.bitcast(hw, bf16), preferred_element_type=f32), HO)

        def mac(br, t, b, pps=range(R)):
            TX, TH = (TXA, THA) if br == "A" else (TXB, THB)
            Z = ZA if br == "A" else ZB
            dvec = PB[2 * t + (br == "B"), 4]
            for pp in pps:
                prow0 = mof((b * R + pp) * PS, 8)
                zrow0 = mof((b * R + pp) * ZS, 16)

                def ld(T, tau):
                    off = HO if T is TH else 0
                    return (T[pl.ds(off + prow0 + tau * 16, 8), :], T[pl.ds(off + prow0 + tau * 16 + 8, 8), :])

                def group(Xg, Hg):
                    Y = [None] * NB
                    if gauss:
                        xs = [Xg[j][0] + Xg[j][1] for j in range(NB)]
                    for m_ in range(NB):
                        hr, hi = Hg[m_]
                        if m_ == 0:
                            hr = hr + dvec
                        else:
                            hr, hi = hr - Hg[m_ - 1][1], hi + Hg[m_ - 1][0]
                        if gauss:
                            hd, he = hi - hr, hr + hi
                        for j in range(NB - m_):
                            xr, xi = Xg[j]
                            i = j + m_
                            if gauss:
                                c3 = (hr * xs[j], hd * xr, he * xi)
                                Y[i] = c3 if Y[i] is None else tuple(u + v for u, v in zip(Y[i], c3))
                            elif Y[i] is None:
                                Y[i] = (xr * hr - xi * hi, xr * hi + xi * hr)
                            else:
                                Y[i] = (Y[i][0] + xr * hr - xi * hi, Y[i][1] + xr * hi + xi * hr)
                    if gauss:
                        Y = [(y[0] - y[2], y[0] + y[1]) for y in Y]
                    return Y

                def stz(tau, zr, zi):
                    Z[pl.ds(zrow0 + tau * 16, 16), :] = jnp.concatenate([zr, zi], axis=0).astype(bf16)

                if R == 2:
                    Ys = []
                    for rp in range(2):
                        sg = (lambda u, v: u + v) if rp == 0 else (lambda u, v: u - v)

                        def bf2(T, j):
                            (a0, a1), (c0, c1) = ld(T, 2 * j), ld(T, 2 * j + 1)
                            return (sg(a0, c0), sg(a1, c1))
                        Ys.append(group([bf2(TX, j) for j in range(NB)], [bf2(TH, j) for j in range(NB)]))
                        if rp == 0 and park:
                            for i in range(NB):
                                MT[pp, 2 * i] = Ys[0][i][0]
                                MT[pp, 2 * i + 1] = Ys[0][i][1]
                    for i in range(NB):
                        a0, a1 = (MT[pp, 2 * i], MT[pp, 2 * i + 1]) if park else Ys[0][i]
                        c0, c1 = Ys[1][i]
                        stz(2 * i, a0 + c0, a1 + c1)
                        stz(2 * i + 1, a0 - c0, a1 - c1)
                else:
                    def pairA(T, j):
                        (r0, i0), (r1, i1), (r2, i2), (r3, i3) = [ld(T, 4 * j + r) for r in range(4)]
                        ar, ai, cr, ci = r0 + r2, i0 + i2, r1 + r3, i1 + i3
                        return [(ar + cr, ai + ci), (ar - cr, ai - ci)]

                    def pairB(T, j):
                        (r0, i0), (r1, i1), (r2, i2), (r3, i3) = [ld(T, 4 * j + r) for r in range(4)]
                        br_, bi, dr, di = r0 - r2, i0 - i2, r1 - r3, i1 - i3
                        return [(br_ + di, bi - dr), (br_ - di, bi + dr)]

                    def pair_mac(pair, emit):
                        X = [pair(TX, j) for j in range(NB)]
                        Y = [[None] * NB for _ in range(2)]
                        prev = None
                        for m_ in range(NB):
                            raw = pair(TH, m_)
                            for g in range(2):
                                hr, hi = raw[g]
                                if m_ == 0:
                                    hr = hr + dvec
                                else:
                                    hr, hi = hr - prev[g][1], hi + prev[g][0]
                                for j in range(NB - m_):
                                    xr, xi = X[j][g]
                                    i = j + m_
                                    if Y[g][i] is None:
                                        Y[g][i] = (xr * hr - xi * hi, xr * hi + xi * hr)
                                    else:
                                        Y[g][i] = (Y[g][i][0] + (xr * hr - xi * hi), Y[g][i][1] + (xr * hi + xi * hr))
                            prev = raw
                            emit(m_, Y[0][m_], Y[1][m_])

                    SD = [None] * NB

                    def emitA(i, y0, y2):
                        sd = (y0[0] + y2[0], y0[1] + y2[1], y0[0] - y2[0], y0[1] - y2[1])
                        if park:
                            for c in range(4):
                                MT[pp, 4 * i + c] = sd[c]
                        else:
                            SD[i] = sd

                    def emitB(i, y1, y3):
                        sr, si, dr, di = [MT[pp, 4 * i + c] for c in range(4)] if park else SD[i]
                        ur, ui = y1[0] + y3[0], y1[1] + y3[1]
                        vr, vi = y1[0] - y3[0], y1[1] - y3[1]
                        stz(4 * i + 0, sr + ur, si + ui)
                        stz(4 * i + 2, sr - ur, si - ui)
                        stz(4 * i + 1, dr - vi, di + vr)
                        stz(4 * i + 3, dr + vi, di - vr)

                    pair_mac(pairA, emitA)
                    pair_mac(pairB, emitB)

        def inv(br, t, b, rs=range(R), cache=None, fin=True):
            cache = {} if cache is None else cache
            Z = ZA if br == "A" else ZB
            for r in rs:
                tau = b * R + r
                zw = jnp.concatenate(
                    [words(Z, (), mof(p * (ZS // 2) + tau * 8, 8), 8) for p in range(16)], axis=0)
                Gm = pltpu.bitcast(G_ref[r], bf16)
                y = jnp.dot(Gm, pltpu.bitcast(zw, bf16), preferred_element_type=f32)
                y0 = mof(tau * M, M)
                (YA if br == "A" else YB)[t, pl.ds(y0, M), :] = y

        def epi(t, b, rs=range(R), cache=None, fin=True, slot=0):
            cache = {} if cache is None else cache
            for r in rs:
                y0 = mof((b * R + r) * M, M)
                if (r >> 1) not in cache:
                    cache[r >> 1] = words(qb, (t,), b * WPB + (r >> 1), M, WS)
                qwd = cache[r >> 1]
                qv = hi(qwd) if r & 1 else lo(qwd)
                g = GT[r & 1, pl.ds(b * WPB + (r >> 1), M, stride=WS), :]
                yb = YB[t, pl.ds(y0, M), :]
                ON[slot, pl.ds(r, M, stride=R), :] = qv * (yb + g * (YA[t, pl.ds(y0, M), :] - yb))
            if fin:
                ob[t, pl.ds(mof(b * R * M, M), R * M), :] = ON[slot].astype(bf16)

        def gate(c):
            r0 = mof(c * M, M)
            accs = [None, None]
            for t in range(NT):
                wd = words(qb, (t,), r0, M)
                wv = bcast(GW[t], M)
                for hf in range(2):
                    x = (hi(wd) if hf else lo(wd)) * wv
                    accs[hf] = x if accs[hf] is None else accs[hf] + x
            for hf in range(2):
                s = jnp.sum(accs[hf], axis=1, keepdims=True)
                GT[hf, pl.ds(r0, M), :] = jnp.broadcast_to(0.5 * jnp.tanh(0.5 * s) + 0.5, (M, CT))

        def scoped(name, fn):
            del name
            fn()

        def loop(n, fn, unr=False):
            if unr:
                for b in range(n):
                    fn(b)
                return

            def body(b, carry):
                fn(b)
                return carry
            lax.fori_loop(0, n, body, 0)

        def phase(fw, mc, iv, mid=None, order=order, static=False, ep=None):
            def body(b, par=None):
                if par is None:
                    par = b % 2 if isinstance(b, int) else lax.rem(b, 2)
                def do_prep(fn):
                    u = 2 * fw[1] + (fw[0] == "B")
                    if isinstance(b, int):
                        un, bn = u + (b + 1) // NB, (b + 1) % NB
                    else:
                        un, bn = u + lax.div(b + 1, NB), lax.rem(b + 1, NB)
                    un = min(un, NU - 1) if isinstance(un, int) else jnp.minimum(un, NU - 1)
                    fn(un, bn, 1 - par)
                caches = {"p": {}, "h": {}, "i": {}}
                toks = []
                for key in order.split("."):
                    if len(key) == 1:
                        toks += [(key, list(range(R)))]
                    else:
                        toks.append((key[0], ["0123abcd".index(c_) % 4 for c_ in key[1:]]))
                for kind, idx in toks:
                    if kind == "x" and fw:
                        fwd_x(fw[0], b, par, idx)
                    elif kind == "h" and fw:
                        fwd_h(fw[0], b, par, idx, caches["h"])
                    elif kind == "m" and mc:
                        mac(*mc, b, idx)
                    elif kind == "i" and iv:
                        inv(*iv, b, idx, caches["i"], fin=False)
                    elif kind == "e" and ep is not None:
                        epi(ep, b)
                    elif kind == "p" and fw:
                        do_prep(lambda un, bn, sl: prep(un, bn, sl, idx, caches["p"]))
                    elif kind == "t" and fw:
                        do_prep(lambda un, bn, sl: prep_h(un, bn, sl, idx))
            if static:
                for b in range(NB):
                    if mid and b == NB - 1:
                        mid()
                    body(b)
            elif mid:
                lax.fori_loop(0, NB // 2, lambda b, c: (body(b), c)[1], 0)
                mid()
                lax.fori_loop(NB // 2, NB, lambda b, c: (body(b), c)[1], 0)
            else:
                loop(NB, body)

        def start_unit(br, t):
            for n in ("h", "k", "v"):
                in_copy(n + br, t).start()

        if True:
            for piece in first[:3]:
                in_copy(*piece).wait()
        for piece in first[6:12]:
            in_copy(*piece).start()
        scoped("prep0", lambda: (prep_h(0, 0, 0), prep(0, 0, 0)))
        small[5].wait()
        if True:
            for b in range(NB):
                if b + 1 < NB:
                    for piece in first[3 * (b + 1):3 * (b + 2)]:
                        in_copy(*piece).wait()
                    if b == 0:
                        for n in ("h", "k", "v"):
                            in_copy(n + "B", 0, 0).start()
                    if b == 1:
                        for blk in range(1, NB):
                            for n in ("h", "k", "v"):
                                in_copy(n + "B", 0, blk).start()
                else:
                    for n in ("h", "k", "v"):
                        in_copy(n + "B", 0, 0).wait()
                    small[6].start()
                    blocks("A", 1, (0, 1), "start")
                fwd_h("A", b, b % 2)
                fwd_x("A", b, b % 2)
                un, bn = (b + 1) // NB, (b + 1) % NB
                prep(un, bn, (b + 1) % 2)
                prep_h(un, bn, (b + 1) % 2)

        def mid_fm():
            blocks("B", 0, (NB - 1,), "wait")
            scoped("w2", lambda: blocks("A", 1, (0,), "wait"))
            scoped("wG", lambda: small[6].wait())
            start_unit("B", 1)

        if True:
            blocks("B", 0, (1, 2), "wait")
        blocks("A", 1, (2, 3), "start")
        scoped("P_fm", lambda: phase(("B", 0), ("A", 0), None, mid=mid_fm, order=o_fm))

        def tile_body(t, carry):
            more = t + 2 < NT

            def mid_b():
                @pl.when(t == 0)
                def _():
                    blocks("A", 1, (NB - 1,), "wait")
                scoped("wB", lambda: wait_unit("B", t + 1))

                @pl.when(t == 0)
                def _():
                    start_unit("B", 2)

                @pl.when(t == 1)
                def _():
                    start_unit("A", 3)

                @pl.when(t == 2)
                def _():
                    start_unit("B", 4)

                @pl.when(t == NT - 2)
                def _():
                    for tt in range(2):
                        for blk in range(NB):
                            out_copy(tt, blk).start()

            def mid_a():
                @pl.when(more)
                def _():
                    scoped("wA", lambda: wait_unit("A", t + 2))

                @pl.when(t == 0)
                def _():
                    for tt in range(NT):
                        in_copy("q", tt).start()

                @pl.when(t == 1)
                def _():
                    start_unit("A", 4)

            @pl.when(t == 0)
            def _():
                scoped("w3", lambda: blocks("A", 1, (1, 2), "wait"))
                start_unit("A", 2)
            scoped("P_B", lambda: phase(("A", t + 1), ("B", t), ("A", t), mid=mid_b, order=o_b))

            @pl.when(t == 1)
            def _():
                if True:
                    for tt in range(NT):
                        in_copy("q", tt).wait()
                start_unit("B", 3)
                scoped("gate", lambda: loop(S // (2 * M) // gu, lambda c: [gate(c * gu + i_) for i_ in range(gu)]))

            ep = jnp.where(t == 0, NT, t - 1)
            scoped("P_A", lambda: phase(("B", t + 1), ("A", t + 1), ("B", t), mid=mid_a, order=o_a, ep=ep))
            return carry

        lax.fori_loop(0, NT - 1, tile_body, 0)
        tl = NT - 1
        for blk in range(NB):
            out_copy(2, blk).start()
        def mid_mi():
            for blk in range(NB // 2):
                out_copy(tl - 1, blk).start()

        scoped("P_mi", lambda: phase(None, ("B", tl), ("A", tl), mid=mid_mi, ep=tl - 1))
        for blk in range(NB // 2, NB):
            out_copy(tl - 1, blk).start()
        if True:
            for b in range(NB):
                inv("B", tl, b)
                if b > 0:
                    epi(tl, b - 1, slot=b % 2)
                    out_copy(tl, b - 1).start()
            epi(tl, NB - 1, slot=NB % 2)
            out_copy(tl, NB - 1).start()
        if True:
            for t in range(NT):
                for blk in range(NB):
                    out_copy(t, blk).wait()

    hbm = pl.BlockSpec(memory_space=pl.ANY)
    vmem = pl.BlockSpec(memory_space=pltpu.VMEM)

    @jax.jit
    def fn(A_q, A_k, A_v, A_shift_k, A_ssm_k, A_ssm_D, B_q, B_k, B_v, B_shift_k, B_ssm_k, B_ssm_D, gate_w):
        del B_q
        out = pl.pallas_call(
            kernel,
            out_shape=jax.ShapeDtypeStruct((S, D), bf16),
            in_specs=[hbm] * 14,
            out_specs=hbm,
            scratch_shapes=[
                pltpu.VMEM((4, D), bf16), pltpu.VMEM((4, D), bf16),
                pltpu.VMEM((D,), bf16), pltpu.VMEM((D,), bf16), pltpu.VMEM((D,), bf16),
                pltpu.VMEM(FXt.shape, u32), pltpu.VMEM(Gt.shape, u32),
                pltpu.VMEM((NT + 1, S // pk, CT), wt),
                pltpu.VMEM((2 * NT, (KPAD + S) // pk, CT), wt),
                pltpu.VMEM((2 * NT, S // pk, CT), wt),
                pltpu.VMEM((2 * NT, CT, S), bf16),
                pltpu.VMEM((NT + 1, S, CT), bf16),
                pltpu.VMEM((2 * NT, 5, 8, CT), f32),
                pltpu.VMEM((NT, 8, CT), f32),
                pltpu.VMEM((2, R * M, CT), bf16),
                pltpu.VMEM((2, 64 * R, CT), u32),
                pltpu.VMEM((16 * PS + 16, CT), f32),
                pltpu.VMEM((16 * PS + 16, CT), f32),
                pltpu.VMEM((16 * PS + 16, CT), f32),
                pltpu.VMEM((16 * PS + 16, CT), f32),
                pltpu.VMEM((16 * ZS, CT), bf16),
                pltpu.VMEM((16 * ZS, CT), bf16),
                pltpu.VMEM((NT + 1, S, CT), f32),
                pltpu.VMEM((NT + 1, S, CT), f32),
                pltpu.VMEM((2, R * M, CT), f32),
                pltpu.VMEM((2, S // 2, CT), f32),
                pltpu.VMEM((R, 16, 8, CT), f32),
                pltpu.SemaphoreType.DMA((7, NT)),
                pltpu.SemaphoreType.DMA((7, 2 * NB)),
                pltpu.SemaphoreType.DMA((NT, NB)),
                pltpu.SemaphoreType.DMA((8,)),
            ],
            compiler_params=pltpu.CompilerParams(vmem_limit_bytes=100 * 1024 * 1024),
            name="h3mix",
        )(A_q.reshape(S, D), A_k.reshape(S, D), A_v.reshape(S, D), A_ssm_k,
          B_k.reshape(S, D), B_v.reshape(S, D), B_ssm_k,
          A_shift_k.T, B_shift_k.T, A_ssm_D, B_ssm_D, gate_w,
          FXt, Gt)
        return out.reshape(1, S, D)

    return fn


pallas_gated_mix__ssm_conv_h3__ssm_conv_h3__prompt_kernel = _build()
```

```python
import jax
import jax.numpy as jnp
import numpy as np
from jax import lax
from jax.experimental import pallas as pl
from jax.experimental.pallas import tpu as pltpu

S = 2048
D = 640
CT = 128
NT = D // CT
M = 128
NTAU = S // M
PS = 264
ZS = 272
KPAD = 16

bf16 = jnp.bfloat16
f32 = jnp.float32
u32 = jnp.uint32


def _bf16_bits(a):
    u = np.ascontiguousarray(a, dtype=np.float32).view(np.uint32).astype(np.uint64)
    r = (u + 0x7FFF + ((u >> 16) & 1)) >> 16
    return r.astype(np.uint32)


def _pack_rows(a):
    b = _bf16_bits(a)
    return (b[0::2] | (b[1::2] << 16)).astype(np.uint32)


def make_tables(R):
    kap = 2 * np.arange(M)
    om = np.pi * (2 * kap + 1) / (256.0 * R)
    m = np.arange(M)
    FX, G = [], []
    for r in range(R):
        ph = np.outer(om, R * m + r)
        F = np.stack([np.cos(ph).reshape(16, 8, M), -np.sin(ph).reshape(16, 8, M)], 1).reshape(2 * M, M)
        FX.append(_pack_rows(F))
        Gm = np.empty((M, 16, 2, 8))
        Gm[:, :, 0, :] = (np.cos(ph).T / (128.0 * R)).reshape(M, 16, 8)
        Gm[:, :, 1, :] = (-np.sin(ph).T / (128.0 * R)).reshape(M, 16, 8)
        G.append(_pack_rows(Gm.reshape(M, 2 * M)))
    return np.stack(FX), np.stack(G)


def mof(x, n):
    return x if isinstance(x, int) else pl.multiple_of(x, n)


def lo(w):
    return pltpu.bitcast(w << 16, f32)


def hi(w):
    return pltpu.bitcast(w & jnp.uint32(0xFFFF0000), f32)


def _build(R=4, order="m0.i0.m1.m3.e.m2.i2.i1.i3", gauss=0, park=1, gu=4,
          o_fm="x.h.m.p.t", o_a="h0.h1.h2.h3.m0.m1.m2.x0.x1.x2.x3.p0.p1.p2.m3.i3.p3.i0.e.i1.i2.t3.t0.t1.t2", o_b="h.m.x.p.i.t"):
    NB = NTAU // R
    WS = R // 2
    WPB = 64 * R
    FXt, Gt = make_tables(R)

    wt, pk = u32, 2

    def words(ref, idx, start, n, stride=1):
        sl = pl.ds(start, n) if stride == 1 else pl.ds(start, n, stride=stride)
        r_ = ref if ref.dtype == u32 else ref.bitcast(u32)
        return r_[(*idx, sl, slice(None))]

    def kernel(q_h, kA_h, vA_h, hA_h, kB_h, vB_h, hB_h,
               skA_h, skB_h, dA_h, dB_h, gw_h,
               FX_h, G_h,
               out_h,
               skA_ref, skB_ref, dA_ref, dB_ref, gw_ref, FX_ref, G_ref,
               qb, kb, vb, hb, ob,
               PB, GW, KV, HT, TXA, THA, TXB, THB, ZA, ZB, YA, YB, ON, GT, MT,
               sem_in, sem_first, sem_out, sem_small):

        def hview(src):
            return src.bitcast(u32)

        RB = R * M

        def in_copy(kind, t, blk=None):
            src_ = {"q": q_h, "kA": kA_h, "vA": vA_h, "kB": kB_h, "vB": vB_h, "hA": hA_h, "hB": hB_h}[kind]
            slot = ["q", "kA", "vA", "hA", "kB", "vB", "hB"].index(kind)
            u = 2 * t + int(kind[-1] == "B")
            sem = sem_in.at[slot, t] if blk is None else sem_first.at[slot, t * NB + blk]
            r0, nr = (0, S) if blk is None else (blk * RB, RB)
            if kind[0] == "h":
                s, d = src_.at[pl.ds(t * CT, CT), pl.ds(r0, nr)], hb.at[u, :, pl.ds(r0, nr)]
            else:
                s = hview(src_).at[pl.ds(r0 // pk, nr // pk), pl.ds(t * CT, CT)]
                off = KPAD if kind[0] == "k" else 0
                dst = {"q": qb.at[t], "k": kb.at[u], "v": vb.at[u]}[kind[0]]
                d = dst.at[pl.ds((off + r0) // pk, nr // pk), :]
            return pltpu.make_async_copy(s, d, sem)

        def out_copy(t, blk):
            rows = pl.ds(blk * RB, RB)
            return pltpu.make_async_copy(ob.at[t, rows, :], out_h.at[rows, pl.ds(t * CT, CT)], sem_out.at[t, blk])

        def blocks(br, t, blks, op):
            for blk in blks:
                for n in ("h", "k", "v"):
                    cp_ = in_copy(n + br, t, blk)
                    cp_.start() if op == "start" else cp_.wait()

        def wait_unit(br, t):
            for n in ("h", "k", "v"):
                in_copy(n + br, t).wait()

        first = [(n + "A", 0, blk) for blk in range(NB) for n in ("h", "k", "v")]
        small = [pltpu.make_async_copy(s_, d_, sem_small.at[i_]) for i_, (s_, d_) in enumerate(
            [(skA_h, skA_ref), (skB_h, skB_ref), (dA_h, dA_ref), (dB_h, dB_ref), (gw_h, gw_ref),
             (FX_h, FX_ref), (G_h, G_ref)])]
        for cp in small[:6]:
            cp.start()
        for piece in first[:6]:
            in_copy(*piece).start()
        YA[NT] = jnp.zeros((S, CT), f32)
        YB[NT] = jnp.zeros((S, CT), f32)
        qb[NT] = jnp.zeros(qb.shape[1:], wt)
        GT[...] = jnp.zeros(GT.shape, f32)
        if True:
            for cp in small[:5]:
                cp.wait()

        skA = skA_ref[...].astype(f32)
        skB = skB_ref[...].astype(f32)
        dA = dA_ref[...].astype(f32)
        dB = dB_ref[...].astype(f32)
        gw = gw_ref[...].astype(f32)
        for t in range(NT):
            sl = slice(t * CT, (t + 1) * CT)
            for u, sk, dd in ((2 * t, skA, dA), (2 * t + 1, skB, dB)):
                for j in range(4):
                    PB[u, j] = jnp.broadcast_to(sk[j:j + 1, sl], (8, CT))
                PB[u, 4] = jnp.broadcast_to(dd[sl].reshape(1, CT), (8, CT))
                kb[u, 0:KPAD // pk, :] = jnp.zeros((KPAD // pk, CT), wt)
            GW[t] = jnp.broadcast_to(gw[sl].reshape(1, CT), (8, CT))
        kpw = KPAD // 2
        NU = 2 * NT
        def bcast(x, n):
            return jnp.broadcast_to(x[None], (n // 8, 8, CT)).reshape(n, CT)

        HO = 16

        def st_tile(T, tau, y, off=0):
            r0 = mof(tau * 16, 16)
            for p in range(16):
                T[pl.ds(off + p * PS + r0, 16), :] = y[p * 16:(p + 1) * 16, :]

        def prep_h(t, b, slot, cs=range(R)):
            for c in cs:
                l0 = mof((b * R + c) * M, M)
                HT[slot, c * 64:(c + 1) * 64, :] = pltpu.bitcast(hb[t, :, pl.ds(l0, M)].T, u32)

        def prep(t, b, slot, rs=range(R), cache=None):
            cache = {} if cache is None else cache
            base = b * WPB
            if "w" not in cache:
                cache["w"] = [bcast(PB[t, j], M) for j in range(4)]
            w = cache["w"]

            def kres(s):
                if s not in cache:
                    wr, hf = s >> 1, s & 1
                    key = ("w", wr)
                    if key not in cache:
                        cache[key] = words(kb, (t,), base + kpw + wr, M, WS)
                    cache[s] = hi(cache[key]) if hf else lo(cache[key])
                return cache[s]

            for r in rs:
                acc = kres(r) * w[0]
                for j in range(1, 4):
                    acc = acc + kres(r - j) * w[j]
                if ("v", r >> 1) not in cache:
                    cache[("v", r >> 1)] = words(vb, (t,), base + (r >> 1), M, WS)
                vw = cache[("v", r >> 1)]
                v = hi(vw) if r & 1 else lo(vw)
                KV[slot, r * M:(r + 1) * M, :] = (acc * v).astype(bf16)

        def fwd_x(br, b, slot, rs=range(R)):
            TX = TXA if br == "A" else TXB
            for r in rs:
                kv = pltpu.bitcast(words(KV, (slot,), r * 64, 64), bf16)
                F = pltpu.bitcast(FX_ref[r], bf16)
                st_tile(TX, b * R + r, jnp.dot(F, kv, preferred_element_type=f32))

        def fwd_h(br, b, slot, rs=range(R), cache=None):
            cache = {} if cache is None else cache
            TH = THA if br == "A" else THB
            for r in rs:
                c = r >> 1
                if c not in cache:
                    cache[c] = (HT[slot, pl.ds(c, 64, stride=2 * WS), :], HT[slot, pl.ds(c + WS, 64, stride=2 * WS), :])
                A, B = cache[c]
                if r & 1 == 0:
                    hw = (A & jnp.uint32(0xFFFF)) | (B << 16)
                else:
                    hw = (A >> 16) | (B & jnp.uint32(0xFFFF0000))
                F = pltpu.bitcast(FX_ref[r], bf16)
                st_tile(TH, b * R + r, jnp.dot(F, pltpu.bitcast(hw, bf16), preferred_element_type=f32), HO)

        def mac(br, t, b, pps=range(R)):
            TX, TH = (TXA, THA) if br == "A" else (TXB, THB)
            Z = ZA if br == "A" else ZB
            dvec = PB[2 * t + (br == "B"), 4]
            for pp in pps:
                prow0 = mof((b * R + pp) * PS, 8)
                zrow0 = mof((b * R + pp) * ZS, 16)

                def ld(T, tau):
                    off = HO if T is TH else 0
                    return (T[pl.ds(off + prow0 + tau * 16, 8), :], T[pl.ds(off + prow0 + tau * 16 + 8, 8), :])

                def group(Xg, Hg):
                    Y = [None] * NB
                    if gauss:
                        xs = [Xg[j][0] + Xg[j][1] for j in range(NB)]
                    for m_ in range(NB):
                        hr, hi = Hg[m_]
                        if m_ == 0:
                            hr = hr + dvec
                        else:
                            hr, hi = hr - Hg[m_ - 1][1], hi + Hg[m_ - 1][0]
                        if gauss:
                            hd, he = hi - hr, hr + hi
                        for j in range(NB - m_):
                            xr, xi = Xg[j]
                            i = j + m_
                            if gauss:
                                c3 = (hr * xs[j], hd * xr, he * xi)
                                Y[i] = c3 if Y[i] is None else tuple(u + v for u, v in zip(Y[i], c3))
                            elif Y[i] is None:
                                Y[i] = (xr * hr - xi * hi, xr * hi + xi * hr)
                            else:
                                Y[i] = (Y[i][0] + xr * hr - xi * hi, Y[i][1] + xr * hi + xi * hr)
                    if gauss:
                        Y = [(y[0] - y[2], y[0] + y[1]) for y in Y]
                    return Y

                def stz(tau, zr, zi):
                    Z[pl.ds(zrow0 + tau * 16, 16), :] = jnp.concatenate([zr, zi], axis=0).astype(bf16)

                if R == 2:
                    Ys = []
                    for rp in range(2):
                        sg = (lambda u, v: u + v) if rp == 0 else (lambda u, v: u - v)

                        def bf2(T, j):
                            (a0, a1), (c0, c1) = ld(T, 2 * j), ld(T, 2 * j + 1)
                            return (sg(a0, c0), sg(a1, c1))
                        Ys.append(group([bf2(TX, j) for j in range(NB)], [bf2(TH, j) for j in range(NB)]))
                        if rp == 0 and park:
                            for i in range(NB):
                                MT[pp, 2 * i] = Ys[0][i][0]
                                MT[pp, 2 * i + 1] = Ys[0][i][1]
                    for i in range(NB):
                        a0, a1 = (MT[pp, 2 * i], MT[pp, 2 * i + 1]) if park else Ys[0][i]
                        c0, c1 = Ys[1][i]
                        stz(2 * i, a0 + c0, a1 + c1)
                        stz(2 * i + 1, a0 - c0, a1 - c1)
                else:
                    def pairA(T, j):
                        (r0, i0), (r1, i1), (r2, i2), (r3, i3) = [ld(T, 4 * j + r) for r in range(4)]
                        ar, ai, cr, ci = r0 + r2, i0 + i2, r1 + r3, i1 + i3
                        return [(ar + cr, ai + ci), (ar - cr, ai - ci)]

                    def pairB(T, j):
                        (r0, i0), (r1, i1), (r2, i2), (r3, i3) = [ld(T, 4 * j + r) for r in range(4)]
                        br_, bi, dr, di = r0 - r2, i0 - i2, r1 - r3, i1 - i3
                        return [(br_ + di, bi - dr), (br_ - di, bi + dr)]

                    def pair_mac(pair, emit):
                        X = [pair(TX, j) for j in range(NB)]
                        Y = [[None] * NB for _ in range(2)]
                        prev = None
                        for m_ in range(NB):
                            raw = pair(TH, m_)
                            for g in range(2):
                                hr, hi = raw[g]
                                if m_ == 0:
                                    hr = hr + dvec
                                else:
                                    hr, hi = hr - prev[g][1], hi + prev[g][0]
                                for j in range(NB - m_):
                                    xr, xi = X[j][g]
                                    i = j + m_
                                    if Y[g][i] is None:
                                        Y[g][i] = (xr * hr - xi * hi, xr * hi + xi * hr)
                                    else:
                                        Y[g][i] = (Y[g][i][0] + (xr * hr - xi * hi), Y[g][i][1] + (xr * hi + xi * hr))
                            prev = raw
                            emit(m_, Y[0][m_], Y[1][m_])

                    SD = [None] * NB

                    def emitA(i, y0, y2):
                        sd = (y0[0] + y2[0], y0[1] + y2[1], y0[0] - y2[0], y0[1] - y2[1])
                        if park:
                            for c in range(4):
                                MT[pp, 4 * i + c] = sd[c]
                        else:
                            SD[i] = sd

                    def emitB(i, y1, y3):
                        sr, si, dr, di = [MT[pp, 4 * i + c] for c in range(4)] if park else SD[i]
                        ur, ui = y1[0] + y3[0], y1[1] + y3[1]
                        vr, vi = y1[0] - y3[0], y1[1] - y3[1]
                        stz(4 * i + 0, sr + ur, si + ui)
                        stz(4 * i + 2, sr - ur, si - ui)
                        stz(4 * i + 1, dr - vi, di + vr)
                        stz(4 * i + 3, dr + vi, di - vr)

                    pair_mac(pairA, emitA)
                    pair_mac(pairB, emitB)

        def inv(br, t, b, rs=range(R), cache=None, fin=True):
            cache = {} if cache is None else cache
            Z = ZA if br == "A" else ZB
            for r in rs:
                tau = b * R + r
                zw = jnp.concatenate(
                    [words(Z, (), mof(p * (ZS // 2) + tau * 8, 8), 8) for p in range(16)], axis=0)
                Gm = pltpu.bitcast(G_ref[r], bf16)
                y = jnp.dot(Gm, pltpu.bitcast(zw, bf16), preferred_element_type=f32)
                y0 = mof(tau * M, M)
                (YA if br == "A" else YB)[t, pl.ds(y0, M), :] = y

        def epi(t, b, rs=range(R), cache=None, fin=True, slot=0):
            cache = {} if cache is None else cache
            for r in rs:
                y0 = mof((b * R + r) * M, M)
                if (r >> 1) not in cache:
                    cache[r >> 1] = words(qb, (t,), b * WPB + (r >> 1), M, WS)
                qwd = cache[r >> 1]
                qv = hi(qwd) if r & 1 else lo(qwd)
                g = GT[r & 1, pl.ds(b * WPB + (r >> 1), M, stride=WS), :]
                yb = YB[t, pl.ds(y0, M), :]
                ON[slot, pl.ds(r, M, stride=R), :] = qv * (yb + g * (YA[t, pl.ds(y0, M), :] - yb))
            if fin:
                ob[t, pl.ds(mof(b * R * M, M), R * M), :] = ON[slot, 0:R * M, :].astype(bf16)

        def gate(c):
            r0 = mof(c * M, M)
            accs = [None, None]
            for t in range(NT):
                wd = words(qb, (t,), r0, M)
                wv = bcast(GW[t], M)
                for hf in range(2):
                    x = (hi(wd) if hf else lo(wd)) * wv
                    accs[hf] = x if accs[hf] is None else accs[hf] + x
            for hf in range(2):
                s = jnp.sum(accs[hf], axis=1, keepdims=True)
                GT[hf, pl.ds(r0, M), :] = jnp.broadcast_to(0.5 * jnp.tanh(0.5 * s) + 0.5, (M, CT))

        def scoped(name, fn):
            del name
            fn()

        def loop(n, fn, unr=False):
            if unr:
                for b in range(n):
                    fn(b)
                return

            def body(b, carry):
                fn(b)
                return carry
            lax.fori_loop(0, n, body, 0)

        def phase(fw, mc, iv, mid=None, order=order, static=False, ep=None):
            def body(b, par=None):
                if par is None:
                    par = b % 2 if isinstance(b, int) else lax.rem(b, 2)
                def do_prep(fn):
                    u = 2 * fw[1] + (fw[0] == "B")
                    if isinstance(b, int):
                        un, bn = u + (b + 1) // NB, (b + 1) % NB
                    else:
                        un, bn = u + lax.div(b + 1, NB), lax.rem(b + 1, NB)
                    un = min(un, NU - 1) if isinstance(un, int) else jnp.minimum(un, NU - 1)
                    fn(un, bn, 1 - par)
                caches = {"p": {}, "h": {}, "i": {}}
                toks = []
                for key in order.split("."):
                    if len(key) == 1:
                        toks += [(key, list(range(R)))]
                    else:
                        toks.append((key[0], ["0123abcd".index(c_) % 4 for c_ in key[1:]]))
                for kind, idx in toks:
                    if kind == "x" and fw:
                        fwd_x(fw[0], b, par, idx)
                    elif kind == "h" and fw:
                        fwd_h(fw[0], b, par, idx, caches["h"])
                    elif kind == "m" and mc:
                        mac(*mc, b, idx)
                    elif kind == "i" and iv:
                        inv(*iv, b, idx, caches["i"], fin=False)
                    elif kind == "e" and ep is not None:
                        epi(ep, b)
                    elif kind == "p" and fw:
                        do_prep(lambda un, bn, sl: prep(un, bn, sl, idx, caches["p"]))
                    elif kind == "t" and fw:
                        do_prep(lambda un, bn, sl: prep_h(un, bn, sl, idx))
            if static:
                for b in range(NB):
                    if mid and b == NB - 1:
                        mid()
                    body(b)
            elif mid:
                lax.fori_loop(0, NB // 2, lambda b, c: (body(b), c)[1], 0)
                mid()
                lax.fori_loop(NB // 2, NB, lambda b, c: (body(b), c)[1], 0)
            else:
                loop(NB, body)

        def start_unit(br, t):
            for n in ("h", "k", "v"):
                in_copy(n + br, t).start()

        if True:
            for piece in first[:3]:
                in_copy(*piece).wait()
        for piece in first[6:12]:
            in_copy(*piece).start()
        scoped("prep0", lambda: (prep_h(0, 0, 0), prep(0, 0, 0)))
        small[5].wait()
        if True:
            for b in range(NB):
                if b + 1 < NB:
                    for piece in first[3 * (b + 1):3 * (b + 2)]:
                        in_copy(*piece).wait()
                    if b == 0:
                        for n in ("h", "k", "v"):
                            in_copy(n + "B", 0, 0).start()
                    if b == 1:
                        for blk in range(1, NB):
                            for n in ("h", "k", "v"):
                                in_copy(n + "B", 0, blk).start()
                else:
                    for n in ("h", "k", "v"):
                        in_copy(n + "B", 0, 0).wait()
                    small[6].start()
                    blocks("A", 1, (0, 1), "start")
                fwd_h("A", b, b % 2)
                fwd_x("A", b, b % 2)
                un, bn = (b + 1) // NB, (b + 1) % NB
                prep(un, bn, (b + 1) % 2)
                prep_h(un, bn, (b + 1) % 2)

        def mid_fm():
            blocks("B", 0, (NB - 1,), "wait")
            scoped("w2", lambda: blocks("A", 1, (0,), "wait"))
            scoped("wG", lambda: small[6].wait())
            start_unit("B", 1)

        if True:
            blocks("B", 0, (1, 2), "wait")
        blocks("A", 1, (2, 3), "start")
        scoped("P_fm", lambda: phase(("B", 0), ("A", 0), None, mid=mid_fm, order=o_fm))

        def tile_body(t, carry):
            more = t + 2 < NT

            def mid_b():
                @pl.when(t == 0)
                def _():
                    blocks("A", 1, (NB - 1,), "wait")
                scoped("wB", lambda: wait_unit("B", t + 1))

                @pl.when(t == 0)
                def _():
                    start_unit("B", 2)

                @pl.when(t == 1)
                def _():
                    start_unit("A", 3)

                @pl.when(t == 2)
                def _():
                    start_unit("B", 4)

                @pl.when(t == NT - 2)
                def _():
                    for tt in range(2):
                        for blk in range(NB):
                            out_copy(tt, blk).start()

            def mid_a():
                @pl.when(more)
                def _():
                    scoped("wA", lambda: wait_unit("A", t + 2))

                @pl.when(t == 0)
                def _():
                    for tt in range(NT):
                        in_copy("q", tt).start()

                @pl.when(t == 1)
                def _():
                    start_unit("A", 4)

            @pl.when(t == 0)
            def _():
                scoped("w3", lambda: blocks("A", 1, (1, 2), "wait"))
                start_unit("A", 2)
            scoped("P_B", lambda: phase(("A", t + 1), ("B", t), ("A", t), mid=mid_b, order=o_b))

            @pl.when(t == 1)
            def _():
                if True:
                    for tt in range(NT):
                        in_copy("q", tt).wait()
                start_unit("B", 3)
                scoped("gate", lambda: loop(S // (2 * M) // gu, lambda c: [gate(c * gu + i_) for i_ in range(gu)]))

            ep = jnp.where(t == 0, NT, t - 1)
            scoped("P_A", lambda: phase(("B", t + 1), ("A", t + 1), ("B", t), mid=mid_a, order=o_a, ep=ep))
            return carry

        lax.fori_loop(0, NT - 1, tile_body, 0)
        tl = NT - 1
        for blk in range(NB):
            out_copy(2, blk).start()
        def mid_mi():
            for blk in range(NB // 2):
                out_copy(tl - 1, blk).start()

        scoped("P_mi", lambda: phase(None, ("B", tl), ("A", tl), mid=mid_mi, ep=tl - 1))
        for blk in range(NB // 2, NB):
            out_copy(tl - 1, blk).start()
        if True:
            for b in range(NB):
                inv("B", tl, b)
                if b > 0:
                    epi(tl, b - 1, slot=b % 2)
                    out_copy(tl, b - 1).start()
            epi(tl, NB - 1, slot=NB % 2)
            out_copy(tl, NB - 1).start()
        if True:
            for t in range(NT):
                for blk in range(NB):
                    out_copy(t, blk).wait()

    hbm = pl.BlockSpec(memory_space=pl.ANY)
    vmem = pl.BlockSpec(memory_space=pltpu.VMEM)

    @jax.jit
    def fn(A_q, A_k, A_v, A_shift_k, A_ssm_k, A_ssm_D, B_q, B_k, B_v, B_shift_k, B_ssm_k, B_ssm_D, gate_w):
        del B_q
        out = pl.pallas_call(
            kernel,
            out_shape=jax.ShapeDtypeStruct((S, D), bf16),
            in_specs=[hbm] * 14,
            out_specs=hbm,
            scratch_shapes=[
                pltpu.VMEM((4, D), bf16), pltpu.VMEM((4, D), bf16),
                pltpu.VMEM((D,), bf16), pltpu.VMEM((D,), bf16), pltpu.VMEM((D,), bf16),
                pltpu.VMEM(FXt.shape, u32), pltpu.VMEM(Gt.shape, u32),
                pltpu.VMEM((NT + 1, S // pk + 32 * (3 - pk), CT), wt),
                pltpu.VMEM((2 * NT, (KPAD + S) // pk + 32 * (3 - pk), CT), wt),
                pltpu.VMEM((2 * NT, S // pk + 32 * (3 - pk), CT), wt),
                pltpu.VMEM((2 * NT, CT, S), bf16),
                pltpu.VMEM((NT + 1, S, CT), bf16),
                pltpu.VMEM((2 * NT, 5, 8, CT), f32),
                pltpu.VMEM((NT, 8, CT), f32),
                pltpu.VMEM((2, R * M, CT), bf16),
                pltpu.VMEM((2, 64 * R + 32, CT), u32),
                pltpu.VMEM((16 * PS + 16, CT), f32),
                pltpu.VMEM((16 * PS + 16, CT), f32),
                pltpu.VMEM((16 * PS + 16, CT), f32),
                pltpu.VMEM((16 * PS + 16, CT), f32),
                pltpu.VMEM((16 * ZS, CT), bf16),
                pltpu.VMEM((16 * ZS, CT), bf16),
                pltpu.VMEM((NT + 1, S, CT), f32),
                pltpu.VMEM((NT + 1, S, CT), f32),
                pltpu.VMEM((2, R * M + 32, CT), f32),
                pltpu.VMEM((2, S // 2 + 32, CT), f32),
                pltpu.VMEM((R, 16, 8, CT), f32),
                pltpu.SemaphoreType.DMA((7, NT)),
                pltpu.SemaphoreType.DMA((7, 2 * NB)),
                pltpu.SemaphoreType.DMA((NT, NB)),
                pltpu.SemaphoreType.DMA((8,)),
            ],
            compiler_params=pltpu.CompilerParams(vmem_limit_bytes=100 * 1024 * 1024),
            name="h3mix",
        )(A_q.reshape(S, D), A_k.reshape(S, D), A_v.reshape(S, D), A_ssm_k,
          B_k.reshape(S, D), B_v.reshape(S, D), B_ssm_k,
          A_shift_k.T, B_shift_k.T, A_ssm_D, B_ssm_D, gate_w,
          FXt, Gt)
        return out.reshape(1, S, D)

    return fn


pallas_gated_mix__ssm_conv_h3__ssm_conv_h3__prompt_kernel = _build()
```
